```python
import jax
import jax.numpy as jnp

def _softmax(x, axis=-1):
    return jax.nn.softmax(x, axis=axis)

def _gelu(x):
    return jax.nn.gelu(x, approximate=True)

def _silu(x):
    return jax.nn.silu(x)

def _sigmoid(x):
    return jax.nn.sigmoid(x)

def _layernorm(x, axis=-1, eps=1e-05):
    m = jnp.mean(x, axis=axis, keepdims=True)
    v = jnp.var(x, axis=axis, keepdims=True)
    return (x - m) / jnp.sqrt(v + eps)

def _scatter_add(tgt, idx, src, axis=0):
    return tgt.at[idx].add(src)

def _segment_sum(src, seg, n):
    return jax.ops.segment_sum(src, seg, n)

class _Rng:

    def __init__(self, key):
        self._k = key

    def _next(self):
        self._k, sub = jax.random.split(self._k)
        return sub

    def normal(self, shape):
        return jax.random.normal(self._next(), shape, dtype=jnp.bfloat16)

    def randint(self, lo, hi, shape):
        return jax.random.randint(self._next(), shape, lo, hi, dtype=jnp.int32)

    def uniform(self, shape, lo=0.0, hi=1.0):
        return jax.random.uniform(self._next(), shape, jnp.bfloat16, lo, hi)

    def permutation(self, n):
        return jax.random.permutation(self._next(), n)
kernel_name = 'concat_heads__memory_aug_recurrent_mem_tr__compressed_kv_cla__prompt'

def setup_inputs():
    _rng = _Rng(jax.random.key(int.from_bytes(__import__("os").urandom(4), "little")))
    _w = lambda a: (lambda t: t.astype(jnp.bfloat16) if jnp.issubdtype(t.dtype, jnp.floating) else t)(jnp.asarray(a))

    def _A_setup():
        B, S, Dm = (1, 2048, 448)
        H, Dh = (16, 256)
        M, seg = (8, 32)
        seg = min(seg, S)
        S = S // seg * seg
        return {'x': _w((lambda *s: _rng.normal(s) * 0.05)(B, S, Dm)), 'mem0': _w((lambda *s: _rng.normal(s) * 0.05)(B, M, Dm)), 'Wq': _w((lambda *s: _rng.normal(s) * 0.05)(Dm, H, Dh) * Dm ** (-0.5)), 'Wk': _w((lambda *s: _rng.normal(s) * 0.05)(Dm, H, Dh) * Dm ** (-0.5)), 'Wv': _w((lambda *s: _rng.normal(s) * 0.05)(Dm, H, Dh) * Dm ** (-0.5)), 'Wo': _w((lambda *s: _rng.normal(s) * 0.05)(H, Dh, Dm) * (H * Dh) ** (-0.5)), 'seg_len': seg}
    _A_in = _A_setup()

    def _B_setup():
        B, H, Sq, Sk, D, M = (1, 16, 2048, 2048, 256, 448)
        Dc = 4 * D
        return {'x': _w((lambda *s: _rng.normal(s) * 0.05)(B, Sq, M)), 'c_kv': _w((lambda *s: _rng.normal(s) * 0.05)(B, Sk, Dc)), 'w_q': _w((lambda *s: _rng.normal(s) * 0.05)(M, H, D) * M ** (-0.5)), 'w_uk': _w((lambda *s: _rng.normal(s) * 0.05)(Dc, H, D) * Dc ** (-0.5)), 'w_uv': _w((lambda *s: _rng.normal(s) * 0.05)(Dc, H, D) * Dc ** (-0.5)), 'w_o': _w((lambda *s: _rng.normal(s) * 0.05)(H, D, M) * (H * D) ** (-0.5))}
    _B_in = _B_setup()
    return {'A_x': _A_in['x'], 'A_mem0': _A_in['mem0'], 'A_Wq': _A_in['Wq'], 'A_Wk': _A_in['Wk'], 'A_Wv': _A_in['Wv'], 'A_Wo': _A_in['Wo'], 'A_seg_len': _A_in['seg_len'], 'B_x': _B_in['x'], 'B_c_kv': _B_in['c_kv'], 'B_w_q': _B_in['w_q'], 'B_w_uk': _B_in['w_uk'], 'B_w_uv': _B_in['w_uv'], 'B_w_o': _B_in['w_o']}

def reference(A_x, A_mem0, A_Wq, A_Wk, A_Wv, A_Wo, A_seg_len, B_x, B_c_kv, B_w_q, B_w_uk, B_w_uv, B_w_o):

    def _A_ref(x, mem0, Wq, Wk, Wv, Wo, seg_len):
        B, S, Dm = x.shape
        H, Dh = (Wq.shape[1], Wq.shape[2])
        M = mem0.shape[1]
        scale = Dh ** (-0.5)
        n_seg = S // seg_len
        L = M + seg_len
        idx = jnp.arange(L)
        mask = (idx[:, None] < M) | (idx[:, None] >= idx[None, :])
        mem = mem0
        outs = []
        for s in range(n_seg):
            xs = x[:, s * seg_len:(s + 1) * seg_len, :].copy()
            h = jnp.concatenate([mem, xs], axis=1)
            q = jnp.einsum('btd,dhe->bhte', h, Wq)
            k = jnp.einsum('btd,dhe->bhte', h, Wk)
            v = jnp.einsum('btd,dhe->bhte', h, Wv)
            scores = jnp.einsum('bhqe,bhke->bhqk', q, k) * scale
            scores = jnp.where(mask[None, None], scores, -1000000000.0)
            p = _softmax(scores, axis=-1)
            o = jnp.einsum('bhqk,bhke->bhqe', p, v)
            o = jnp.einsum('bhte,hed->btd', o, Wo)
            mem = o[:, :M, :].copy()
            outs.append(o[:, M:, :])
        return jnp.concatenate(outs, axis=1)

    def _B_ref(x, c_kv, w_q, w_uk, w_uv, w_o):
        B, Sq, M = (x.shape[0], x.shape[1], x.shape[2])
        Sk = c_kv.shape[1]
        H, D = (w_q.shape[1], w_q.shape[2])
        q = jnp.einsum('bqm,mhd->bhqd', x, w_q)
        k = jnp.einsum('bkc,chd->bhkd', c_kv, w_uk)
        v = jnp.einsum('bkc,chd->bhkd', c_kv, w_uv)
        scores = jnp.einsum('bhqd,bhkd->bhqk', q, k) * D ** (-0.5)
        off = Sk - Sq
        qi = jnp.arange(Sq)[:, None]
        kj = jnp.arange(Sk)[None, :]
        cmask = kj <= qi + off
        scores = jnp.where(cmask[None, None], scores, -1000000000.0)
        p = _softmax(scores, axis=-1)
        ctx = jnp.einsum('bhqk,bhkd->bhqd', p, v)
        return jnp.einsum('bhqd,hdm->bqm', ctx, w_o)
    a = _A_ref(A_x, A_mem0, A_Wq, A_Wk, A_Wv, A_Wo, A_seg_len)
    b = _B_ref(B_x, B_c_kv, B_w_q, B_w_uk, B_w_uv, B_w_o)
    return jnp.concatenate([a, b], axis=-1)
```

```python
import functools, os

import jax
import jax.numpy as jnp
import numpy as np
from jax.experimental import pallas as pl
from jax.experimental.pallas import tpu as pltpu

_LOG2E = float(np.log2(np.e))
_NN = (((1,), (0,)), ((), ()))
_NT = (((1,), (1,)), ((), ()))
_HI = np.uint32(0xFFFF0000)
E = lambda k, d: type(d)(os.environ.get(k, d))
NSTEP = E("NSTEP", 64); NHEAD = E("NHEAD", 16); AORD = E("AORD", 4); LAG1 = E("LAG1", 1); LAG2 = E("LAG2", 1)


def _dot(a, b, dims=_NN):
    return jax.lax.dot_general(a, b, dims, preferred_element_type=jnp.float32)


def _kernel(axt_hbm, am_hbm, awq_hbm, awk_hbm, awv_hbm, awot_hbm,
            bxt_hbm, bc_hbm, bwq_hbm, bwk_hbm, bwv_hbm, bwot_hbm,
            out_hbm,
            xt_raw, ax_v, am_v, aw_raw, aw_v, awot_raw, awo_v,
            bx_v, bc_v, bw_raw, bw_v, bwot_v,
            q_v, k_v, v_v, ctx_v, out_v,
            sem_in, sem_bw, sem_aw, sem_out,
            *, S, Dm, H, Dh, M, SEG, Sq, Dc, TQ, OUT_STEPS):
    HP = H // 2
    n_seg = S // SEG
    L = M + SEG

    bwq_u = bwq_hbm.bitcast(jnp.uint32)
    bwk_u = bwk_hbm.bitcast(jnp.uint32)
    bwv_u = bwv_hbm.bitcast(jnp.uint32)
    aw_u = [r.bitcast(jnp.uint32) for r in (awq_hbm, awk_hbm, awv_hbm)]

    def bw_copies(j, slot):
        return [
            pltpu.make_async_copy(bwq_u.at[:, j, :], bw_raw.at[slot, pl.ds(0, Dm)], sem_bw.at[slot, 0]),
            pltpu.make_async_copy(bwk_u.at[:, j, :], bw_raw.at[slot, pl.ds(Dm, Dc)], sem_bw.at[slot, 1]),
            pltpu.make_async_copy(bwv_u.at[:, j, :], bw_raw.at[slot, pl.ds(Dm + Dc, Dc)], sem_bw.at[slot, 2]),
        ]

    def aw_copies(j):
        return [pltpu.make_async_copy(aw_u[t].at[:, j, :], aw_raw.at[t], sem_aw.at[t]) for t in range(3)]

    c_bx = pltpu.make_async_copy(bxt_hbm, xt_raw.at[0], sem_in.at[0])
    c_bc = pltpu.make_async_copy(bc_hbm, bc_v, sem_in.at[1])
    c_bwo = pltpu.make_async_copy(bwot_hbm, bwot_v, sem_in.at[2])
    c_ax = pltpu.make_async_copy(axt_hbm, xt_raw.at[1], sem_in.at[3])
    c_am = pltpu.make_async_copy(am_hbm, am_v, sem_in.at[4])
    c_awo = pltpu.make_async_copy(awot_hbm, awot_raw, sem_in.at[5])

    c_bx.start()
    for c in bw_copies(0, 0):
        c.start()
    c_bc.start()
    c_ax.start()
    c_am.start()
    c_bwo.start()
    c_awo.start()
    c_bx.wait()

    def xpose_x(src, dst):
        def body(i, carry):
            r0 = pl.multiple_of(i * 256, 256)
            dst[pl.ds(r0, 256), :] = src[:, pl.ds(r0, 256)].astype(jnp.float32).T.astype(dst.dtype)
            return carry
        jax.lax.fori_loop(0, S // 256, body, 0)

    xpose_x(xt_raw.at[0], bx_v)
    c_bc.wait()

    b_scale = float(Dh) ** -0.5 * _LOG2E
    row = jax.lax.broadcasted_iota(jnp.int32, (TQ, TQ), 0)
    col = jax.lax.broadcasted_iota(jnp.int32, (TQ, TQ), 1)

    def head_body(h, carry):
        j = h // 2
        odd = h % 2
        slot = j % 2

        @pl.when(odd == 0)
        def _():
            for c in bw_copies(j, slot):
                c.wait()

            @pl.when(j + 1 < NHEAD // 2)
            def _():
                for c in bw_copies(j + 1, 1 - slot):
                    c.start()

            for c in aw_copies(j):
                c.start()

        @pl.when(odd == 1)
        def _():
            for c in aw_copies(j):
                c.wait()
            for t in range(3):
                u = aw_raw[t]
                aw_v[t * H + 2 * j] = pltpu.bitcast(u << 16, jnp.float32)
                aw_v[t * H + 2 * j + 1] = pltpu.bitcast(u & _HI, jnp.float32)

        sh = (16 * (1 - odd)).astype(jnp.uint32)
        bw_v[...] = pltpu.bitcast((bw_raw[slot] << sh) & _HI, jnp.float32).astype(jnp.bfloat16)

        q_v[...] = (_dot(bx_v[...], bw_v[pl.ds(0, Dm)]) * b_scale).astype(jnp.bfloat16)
        k_v[...] = _dot(bc_v[...], bw_v[pl.ds(Dm, Dc)]).astype(jnp.bfloat16)
        v_v[...] = _dot(bc_v[...], bw_v[pl.ds(Dm + Dc, Dc)]).astype(jnp.bfloat16)

        for i in range(Sq // TQ):
            r0 = i * TQ
            q = q_v[pl.ds(r0, TQ)]
            sd = jnp.where(col <= row, _dot(q, k_v[pl.ds(r0, TQ)], _NT), -1e30)
            m = jnp.max(sd, axis=1, keepdims=True)
            if i > 0:
                so = _dot(q, k_v[pl.ds(0, r0)], _NT)
                m = jnp.maximum(m, jnp.max(so, axis=1, keepdims=True))
            pd = jnp.exp2(sd - m)
            l = jnp.sum(pd, axis=1, keepdims=True)
            o = _dot(pd.astype(jnp.bfloat16), v_v[pl.ds(r0, TQ)])
            if i > 0:
                po = jnp.exp2(so - m)
                l = l + jnp.sum(po, axis=1, keepdims=True)
                o = o + _dot(po.astype(jnp.bfloat16), v_v[pl.ds(0, r0)])
            ctx_v[h, pl.ds(r0, TQ)] = (o * (1.0 / l)).astype(jnp.bfloat16)
        return carry

    jax.lax.fori_loop(0, NHEAD, head_body, 0)

    c_bwo.wait()
    c_ax.wait()
    c_am.wait()
    c_awo.wait()

    def bout_body(i, carry):
        r0 = pl.multiple_of(i * TQ, TQ)
        acc = _dot(bwot_v[0], ctx_v[0, pl.ds(r0, TQ)], _NT)
        for h in range(1, H):
            acc = acc + _dot(bwot_v[h], ctx_v[h, pl.ds(r0, TQ)], _NT)
        out_v[pl.ds(r0, TQ), pl.ds(Dm, Dm)] = acc.T.astype(jnp.bfloat16)
        ax_v[pl.ds(r0, TQ), :] = xt_raw[1, :, pl.ds(r0, TQ)].astype(jnp.float32).T
        for hh in range(H // (Sq // TQ)):
            hx = i * (H // (Sq // TQ)) + hh
            awo_v[hx] = awot_raw[hx].astype(jnp.float32).T
        return carry

    jax.lax.fori_loop(0, Sq // TQ, bout_body, 0)

    a_scale = float(Dh) ** -0.5 * _LOG2E
    arow = jax.lax.broadcasted_iota(jnp.int32, (L, L), 0)
    acol = jax.lax.broadcasted_iota(jnp.int32, (L, L), 1)
    amask = (arow < M) | (arow >= acol)
    OUT_ROWS = OUT_STEPS * SEG

    def out_copy(g):
        r0 = pl.multiple_of(g * OUT_ROWS, OUT_ROWS)
        return pltpu.make_async_copy(out_v.at[pl.ds(r0, OUT_ROWS)], out_hbm.at[pl.ds(r0, OUT_ROWS)], sem_out.at[g % 2])

    def seg_body(s, mem):
        r0 = pl.multiple_of(s * SEG, SEG)
        hin = jnp.concatenate([mem, ax_v[pl.ds(r0, SEG)]], axis=0)
        q, k, v, sc, p, o = ({} for _ in range(6))
        acc = [None]

        def QK(h):
            q[h] = _dot(hin, aw_v[h])
            k[h] = _dot(hin, aw_v[H + h])

        def V(h):
            v[h] = _dot(hin, aw_v[2 * H + h])

        def SC(h):
            sc[h] = _dot(q[h], k[h], _NT)

        def SM(h):
            x = jnp.where(amask, sc[h] * a_scale, -1e30)
            e = jnp.exp2(x - jnp.max(x, axis=1, keepdims=True))
            p[h] = e * (1.0 / jnp.sum(e, axis=1, keepdims=True))

        def PV(h):
            o[h] = _dot(p[h], v[h])

        def OUT(h):
            t = _dot(o[h], awo_v[h])
            acc[0] = t if acc[0] is None else acc[0] + t

        def run(stages, n):
            mx = max(l for _, l in stages)
            for t in range(n + mx):
                for fn, l in stages:
                    if 0 <= t - l < n:
                        fn(t - l)

        if AORD == 1:
            run([(QK, 0), (SC, 1), (V, 0), (SM, 1), (PV, 2), (OUT, 3)], H)
        elif AORD == 2:
            run([(QK, 0), (SC, LAG1), (SM, LAG1 + LAG2)], H)
            run([(V, 0), (PV, 1)], H)
            run([(OUT, 0)], H)
        elif AORD == 3:
            run([(QK, 0), (SC, LAG1)], H)
            run([(V, 0), (SM, 0), (PV, 1)], H)
            run([(OUT, 0)], H)
        elif AORD == 4:
            run([(QK, 0), (SC, LAG1), (SM, LAG1 + LAG2)], H)
            run([(V, 0), (PV, 1), (OUT, 2)], H)
        accb = acc[0].astype(jnp.bfloat16)
        out_v[pl.ds(r0, SEG), pl.ds(0, Dm)] = acc[0][M:].astype(jnp.bfloat16)

        @pl.when((s + 1) % OUT_STEPS == 0)
        def _():
            g = s // OUT_STEPS

            @pl.when(g >= 2)
            def _():
                out_copy(g - 2).wait()

            out_copy(g).start()

        return acc[0][:M].astype(jnp.bfloat16).astype(jnp.float32)

    jax.lax.fori_loop(0, NSTEP, seg_body, am_v[...].astype(jnp.float32))
    n_out = NSTEP // OUT_STEPS
    for g in range(max(n_out - 2, 0), n_out):
        out_copy(g).wait()


@functools.partial(jax.jit, static_argnames=("A_seg_len",))
def pallas_concat_heads__memory_aug_recurrent_mem_tr__compressed_kv_cla__prompt_kernel(
    A_x, A_mem0, A_Wq, A_Wk, A_Wv, A_Wo, A_seg_len,
    B_x, B_c_kv, B_w_q, B_w_uk, B_w_uv, B_w_o,
):
    _, S, Dm = A_x.shape
    _, H, Dh = A_Wq.shape
    M = A_mem0.shape[1]
    SEG = int(A_seg_len)
    _, Sq, Dc = B_c_kv.shape
    TQ = 256
    OUT_STEPS = 8
    bf16, f32, u32 = jnp.bfloat16, jnp.float32, jnp.uint32
    kern = functools.partial(_kernel, S=S, Dm=Dm, H=H, Dh=Dh, M=M, SEG=SEG, Sq=Sq, Dc=Dc, TQ=TQ,
                             OUT_STEPS=OUT_STEPS)
    out = pl.pallas_call(
        kern,
        out_shape=jax.ShapeDtypeStruct((S, 2 * Dm), bf16),
        in_specs=[pl.BlockSpec(memory_space=pl.ANY)] * 12,
        out_specs=pl.BlockSpec(memory_space=pl.ANY),
        scratch_shapes=[
            pltpu.VMEM((2, Dm, S), bf16),
            pltpu.VMEM((S, Dm), f32),
            pltpu.VMEM((M, Dm), bf16),
            pltpu.VMEM((3, Dm, Dh), u32),
            pltpu.VMEM((3 * H, Dm, Dh), f32),
            pltpu.VMEM((H, Dm, Dh), bf16),
            pltpu.VMEM((H, Dh, Dm), f32),
            pltpu.VMEM((Sq, Dm), bf16),
            pltpu.VMEM((Sq, Dc), bf16),
            pltpu.VMEM((2, Dm + 2 * Dc, Dh), u32),
            pltpu.VMEM((Dm + 2 * Dc, Dh), bf16),
            pltpu.VMEM((H, Dm, Dh), bf16),
            pltpu.VMEM((Sq, Dh), bf16),
            pltpu.VMEM((Sq, Dh), bf16),
            pltpu.VMEM((Sq, Dh), bf16),
            pltpu.VMEM((H, Sq, Dh), bf16),
            pltpu.VMEM((S, 2 * Dm), bf16),
            pltpu.SemaphoreType.DMA((6,)),
            pltpu.SemaphoreType.DMA((2, 3)),
            pltpu.SemaphoreType.DMA((3,)),
            pltpu.SemaphoreType.DMA((2,)),
        ],
        compiler_params=pltpu.CompilerParams(vmem_limit_bytes=120 * 2**20),
    )(A_x.reshape(S, Dm).T, A_mem0.reshape(M, Dm), A_Wq, A_Wk, A_Wv, A_Wo.transpose(0, 2, 1),
      B_x.reshape(Sq, Dm).T, B_c_kv.reshape(Sq, Dc), B_w_q, B_w_uk, B_w_uv, B_w_o.transpose(0, 2, 1))
    return out.reshape(1, S, 2 * Dm)
```

```python
import functools

import jax
import jax.numpy as jnp
import numpy as np
from jax.experimental import pallas as pl
from jax.experimental.pallas import tpu as pltpu

_LOG2E = float(np.log2(np.e))
_NN = (((1,), (0,)), ((), ()))
_NT = (((1,), (1,)), ((), ()))
_HI = np.uint32(0xFFFF0000)
_NEG = -1e30


def _dot(a, b, dims=_NN):
    return jax.lax.dot_general(a, b, dims, preferred_element_type=jnp.float32)


def _merge(*lists):
    items = []
    for li, l in enumerate(lists):
        total = float(sum(c for c, _ in l))
        done = 0.0
        for k, (c, f) in enumerate(l):
            items.append(((done + 0.5 * c) / total, li, k, c, f))
            done += c
    items.sort(key=lambda t: t[:3])
    return [(c, f) for _, _, _, c, f in items]


def _run(prog):
    for _, f in prog:
        f()


def _kernel(axt_hbm, am_hbm, awq_hbm, awk_hbm, awv_hbm, awot_hbm,
            bxt_hbm, bc_hbm, bwq_hbm, bwk_hbm, bwv_hbm, bwot_hbm,
            out_hbm,
            xt_raw, ax_v, am_v, aw_raw, aw_v, awot_raw, awo_v,
            bx_v, bc_v, bw_raw, bw_v, bwot_v,
            q_v, k_v, v_v, ctx_v, out_v, acc_v,
            sem_in, sem_bw, sem_aw, sem_out,
            *, S, Dm, H, Dh, M, SEG, Sq, Dc, TQ):
    HP = H // 2
    L = M + SEG
    NQ = Sq // TQ
    HT = TQ // 2
    n_seg = S // SEG
    OT = 128
    OG = n_seg // (Sq // OT)
    OH = H // OG
    scale = float(Dh) ** -0.5 * _LOG2E

    bwq_u = bwq_hbm.bitcast(jnp.uint32)
    bwk_u = bwk_hbm.bitcast(jnp.uint32)
    bwv_u = bwv_hbm.bitcast(jnp.uint32)
    aw_u = [r.bitcast(jnp.uint32) for r in (awq_hbm, awk_hbm, awv_hbm)]

    def bw_copies(j, slot):
        return [
            pltpu.make_async_copy(bwk_u.at[:, j, :], bw_raw.at[slot, pl.ds(Dm, Dc)], sem_bw.at[slot, 1]),
            pltpu.make_async_copy(bwv_u.at[:, j, :], bw_raw.at[slot, pl.ds(Dm + Dc, Dc)], sem_bw.at[slot, 2]),
            pltpu.make_async_copy(bwq_u.at[:, j, :], bw_raw.at[slot, pl.ds(0, Dm)], sem_bw.at[slot, 0]),
        ]

    def aw_copies(j, slot):
        return [pltpu.make_async_copy(aw_u[t].at[:, j, :], aw_raw.at[slot, t], sem_aw.at[slot, t]) for t in range(3)]

    c_bx = pltpu.make_async_copy(bxt_hbm, xt_raw.at[0], sem_in.at[0])
    c_bc = pltpu.make_async_copy(bc_hbm, bc_v, sem_in.at[5])
    c_bwo = pltpu.make_async_copy(bwot_hbm, bwot_v, sem_in.at[1])
    c_ax = pltpu.make_async_copy(axt_hbm, xt_raw.at[1], sem_in.at[2])
    c_am = pltpu.make_async_copy(am_hbm, am_v, sem_in.at[3])
    c_awo = pltpu.make_async_copy(awot_hbm, awot_raw, sem_in.at[4])

    def unpack_b(h, lo=0, hi=Dm + 2 * Dc, step=416):
        if isinstance(h, int):
            sh = np.uint32(16 * (1 - h % 2))
        else:
            sh = (16 * (1 - h % 2)).astype(jnp.uint32)
        slot = (h // 2) % 2
        out = []
        for r0 in range(lo, hi, step):
            def f(r0=r0):
                u = (bw_raw[slot, pl.ds(r0, step)] << sh) & _HI
                bw_v[pl.ds(r0, step)] = pltpu.bitcast(u, jnp.float32).astype(jnp.bfloat16)
            out.append((1, f))
        return out

    def proj_q(r0, n):
        q_v[pl.ds(r0, n)] = (_dot(bx_v[pl.ds(r0, n)], bw_v[pl.ds(0, Dm)]) * scale).astype(jnp.bfloat16)

    def proj_k(r0, n):
        k_v[pl.ds(r0, n)] = _dot(bc_v[pl.ds(r0, n)], bw_v[pl.ds(Dm, Dc)]).astype(jnp.bfloat16)

    def proj_v(r0, n):
        v_v[pl.ds(r0, n)] = _dot(bc_v[pl.ds(r0, n)], bw_v[pl.ds(Dm + Dc, Dc)]).astype(jnp.bfloat16)

    def b_proj(n):
        return ([(2 * n, functools.partial(proj_q, r0, n)) for r0 in range(0, Sq, n)]
                + [(4 * n, functools.partial(proj_k, r0, n)) for r0 in range(0, Sq, n)]
                + [(4 * n, functools.partial(proj_v, r0, n)) for r0 in range(0, Sq, n)])

    tri = jax.lax.broadcasted_iota(jnp.int32, (HT, HT), 1) <= jax.lax.broadcasted_iota(jnp.int32, (HT, HT), 0)

    def b_attn(h):
        st = {}

        def scores(i):
            r0 = i * TQ
            d = st[i] = {"s": {}}

            def diag():
                q = q_v[pl.ds(r0, TQ)]
                sl = _dot(q, k_v[pl.ds(r0, HT)], _NT)
                sl = jnp.concatenate([jnp.where(tri, sl[:HT], _NEG), sl[HT:]], axis=0)
                sr = jnp.where(tri, _dot(q[HT:], k_v[pl.ds(r0 + HT, HT)], _NT), _NEG)
                d["sl"], d["sr"] = sl, sr
                d["m"] = jnp.concatenate([sl[:HT], jnp.maximum(sl[HT:], sr)], axis=0)

            def off(c):
                s = _dot(q_v[pl.ds(r0, TQ)], k_v[pl.ds(c * TQ, TQ)], _NT)
                d["s"][c] = s
                d["m"] = jnp.maximum(d["m"], jnp.maximum(s[:, :HT], s[:, HT:]))

            def fin():
                d["m"] = jnp.max(d["m"], axis=1, keepdims=True)

            return ([(3 * TQ // 4, diag)] + [(TQ, functools.partial(off, c)) for c in range(i)] + [(1, fin)])

        def values(i):
            r0 = i * TQ

            def diag():
                d = st[i]
                m = d["m"]
                pl_ = jnp.exp2(d["sl"] - m)
                pr = jnp.exp2(d["sr"] - m[HT:])
                d["l"] = jnp.concatenate([pl_[:HT], pl_[HT:] + pr], axis=0)
                o = _dot(pl_.astype(jnp.bfloat16), v_v[pl.ds(r0, HT)])
                ob = _dot(pr.astype(jnp.bfloat16), v_v[pl.ds(r0 + HT, HT)])
                d["o"] = jnp.concatenate([o[:HT], o[HT:] + ob], axis=0)

            def off(c):
                d = st[i]
                p = jnp.exp2(d["s"][c] - d["m"])
                d["l"] = d["l"] + (p[:, :HT] + p[:, HT:])
                d["o"] = d["o"] + _dot(p.astype(jnp.bfloat16), v_v[pl.ds(c * TQ, TQ)])

            def fin():
                d = st[i]
                l = jnp.sum(d["l"], axis=1, keepdims=True)
                ctx_v[h, pl.ds(r0, TQ)] = (d["o"] * (1.0 / l)).astype(jnp.bfloat16)

            return ([(3 * TQ // 4, diag)] + [(TQ, functools.partial(off, c)) for c in range(i)] + [(1, fin)])

        prog = []
        for t in range(NQ + 1):
            ls = []
            if t < NQ:
                ls.append(scores(NQ - 1 - t))
            if t >= 1:
                ls.append(values(NQ - t))
            prog += _merge(*ls)
        return prog

    def a_prep(h):
        sh = (16 * (1 - h % 2)).astype(jnp.uint32)
        slot = (h // 2) % 2
        out = []
        for t in range(3):
            def f(t=t):
                aw_v[t * H + h] = pltpu.bitcast((aw_raw[slot, t] << sh) & _HI, jnp.float32)
            out.append((1, f))

        def fo():
            awo_v[h] = awot_raw[h].astype(jnp.float32).T

        def fx():
            n = S // H
            r0 = pl.multiple_of(h * n, n)
            ax_v[pl.ds(r0, n), :] = xt_raw[1, :, pl.ds(r0, n)].astype(jnp.float32).T

        return out + [(1, fo), (1, fx)]

    arow = jax.lax.broadcasted_iota(jnp.int32, (L, L), 0)
    acol = jax.lax.broadcasted_iota(jnp.int32, (L, L), 1)
    amask = (arow < M) | (arow >= acol)

    def a_step(s, state):
        r0 = pl.multiple_of(s * SEG, SEG)
        q, k, v, sc, p, o = ({} for _ in range(6))
        d = {}

        def start():
            d["h"] = jnp.concatenate([state["mem"], ax_v[pl.ds(r0, SEG)]], axis=0)

        def QK(h):
            q[h] = _dot(d["h"], aw_v[h])
            k[h] = _dot(d["h"], aw_v[H + h])

        def V(h):
            v[h] = _dot(d["h"], aw_v[2 * H + h])

        def SC(h):
            sc[h] = _dot(q[h], k[h], _NT)

        def SM(h):
            x = jnp.where(amask, sc[h] * scale, _NEG)
            e = jnp.exp2(x - jnp.max(x, axis=1, keepdims=True))
            p[h] = e * (1.0 / jnp.sum(e, axis=1, keepdims=True))

        def PV(h):
            o[h] = _dot(p[h], v[h])

        def OUT(h):
            t = _dot(o[h], awo_v[h])
            d["acc"] = t if h == 0 else d["acc"] + t

        def finish():
            out_v[pl.ds(r0, SEG), pl.ds(0, Dm)] = d["acc"][M:].astype(jnp.bfloat16)
            state["mem"] = d["acc"][:M].astype(jnp.bfloat16).astype(jnp.float32)

        prog = [(60, start)]
        order = ([(QK, 0, 160), (SC, 1, 20), (SM, 2, 1)], [(V, 0, 80), (PV, 1, 20), (OUT, 2, 80)])
        for stages in order:
            for t in range(H + stages[-1][1]):
                for fn, lag, c in stages:
                    if 0 <= t - lag < H:
                        prog.append((c, functools.partial(fn, t - lag)))
        prog.append((60, finish))
        return prog

    def b_out(s):
        g = s // OG
        r0 = pl.multiple_of(g * OT, OT)
        h0 = (s % OG) * OH
        d = {}

        def part(u):
            t = _dot(bwot_v[h0 + u], ctx_v[h0 + u, pl.ds(r0, OT)], _NT)
            d["acc"] = (jnp.where(s % OG == 0, 0.0, acc_v[...]) if u == 0 else d["acc"]) + t

        def fin():
            acc_v[...] = d["acc"]
            out_v[pl.ds(r0, OT), pl.ds(Dm, Dm)] = d["acc"].T.astype(jnp.bfloat16)

        return [(Dm // 2, functools.partial(part, u)) for u in range(OH)] + [(1, fin)]

    def out_copy(g):
        r0 = pl.multiple_of(g * OT, OT)
        return pltpu.make_async_copy(out_v.at[pl.ds(r0, OT)], out_hbm.at[pl.ds(r0, OT)], sem_out.at[g])

    w0 = bw_copies(0, 0)
    c_bx.start()
    w0[2].start()
    w0[0].start()
    c_bc.start()
    w0[1].start()
    for c in aw_copies(0, 0):
        c.start()
    c_ax.start()
    c_awo.start()
    c_am.start()
    c_bwo.start()
    c_bx.wait()

    def xpose_body(i, carry):
        r0 = pl.multiple_of(i * TQ, TQ)
        bx_v[pl.ds(r0, TQ), :] = xt_raw[0, :, pl.ds(r0, TQ)].astype(jnp.float32).T.astype(jnp.bfloat16)
        return carry

    jax.lax.fori_loop(0, NQ, xpose_body, 0)
    w0[2].wait()
    _run(unpack_b(0, 0, Dm, Dm))

    def head_body(h, carry):
        j = h // 2
        proj_q(0, Sq)

        @pl.when(h == 0)
        def _():
            w0[0].wait()
            w0[1].wait()

            def body(i, carry):
                r0 = pl.multiple_of(Dm + i * 128, 64)
                bw_v[pl.ds(r0, 128)] = pltpu.bitcast(bw_raw[0, pl.ds(r0, 128)] << 16, jnp.float32).astype(jnp.bfloat16)
                return carry

            jax.lax.fori_loop(0, 2 * Dc // 128, body, 0)
            c_bc.wait()

        @pl.when((h % 2 == 0) & (j + 1 < HP))
        def _():
            for c in bw_copies(j + 1, (j + 1) % 2) + aw_copies(j + 1, (j + 1) % 2):
                c.start()

        @pl.when((h % 2 == 1) & (j + 1 < HP))
        def _():
            for c in bw_copies(j + 1, (j + 1) % 2):
                c.wait()

        proj_k(0, Sq)
        proj_v(0, Sq)

        @pl.when(h % 2 == 0)
        def _():
            for c in aw_copies(j, j % 2):
                c.wait()

        @pl.when(h == 0)
        def _():
            c_ax.wait()
            c_awo.wait()

        _run(_merge(b_attn(h), unpack_b(jnp.minimum(h + 1, H - 1)) + a_prep(h)))
        return carry

    jax.lax.fori_loop(0, H, head_body, 0)
    c_am.wait()
    c_bwo.wait()
    acc_v[...] = jnp.zeros_like(acc_v)

    def seg_body(s, mem):
        state = {"mem": mem}
        _run(b_out(s) + a_step(s, state))

        @pl.when(s % OG == OG - 1)
        def _():
            out_copy(s // OG).start()

        return state["mem"]

    jax.lax.fori_loop(0, n_seg, seg_body, am_v[...].astype(jnp.float32))
    for g in range(Sq // OT):
        out_copy(g).wait()


@functools.partial(jax.jit, static_argnames=("A_seg_len",))
def pallas_concat_heads__memory_aug_recurrent_mem_tr__compressed_kv_cla__prompt_kernel(
    A_x, A_mem0, A_Wq, A_Wk, A_Wv, A_Wo, A_seg_len,
    B_x, B_c_kv, B_w_q, B_w_uk, B_w_uv, B_w_o,
):
    _, S, Dm = A_x.shape
    _, H, Dh = A_Wq.shape
    M = A_mem0.shape[1]
    SEG = int(A_seg_len)
    _, Sq, Dc = B_c_kv.shape
    TQ = 256
    bf16, f32, u32 = jnp.bfloat16, jnp.float32, jnp.uint32
    kern = functools.partial(_kernel, S=S, Dm=Dm, H=H, Dh=Dh, M=M, SEG=SEG, Sq=Sq, Dc=Dc, TQ=TQ)
    out = pl.pallas_call(
        kern,
        out_shape=jax.ShapeDtypeStruct((S, 2 * Dm), bf16),
        in_specs=[pl.BlockSpec(memory_space=pltpu.HBM)] * 12,
        out_specs=pl.BlockSpec(memory_space=pltpu.HBM),
        scratch_shapes=[
            pltpu.VMEM((2, Dm, S), bf16),
            pltpu.VMEM((S, Dm), f32),
            pltpu.VMEM((M, Dm), bf16),
            pltpu.VMEM((2, 3, Dm, Dh), u32),
            pltpu.VMEM((3 * H, Dm, Dh), f32),
            pltpu.VMEM((H, Dm, Dh), bf16),
            pltpu.VMEM((H, Dh, Dm), f32),
            pltpu.VMEM((Sq, Dm), bf16),
            pltpu.VMEM((Sq, Dc), bf16),
            pltpu.VMEM((2, Dm + 2 * Dc, Dh), u32),
            pltpu.VMEM((Dm + 2 * Dc, Dh), bf16),
            pltpu.VMEM((H, Dm, Dh), bf16),
            pltpu.VMEM((Sq, Dh), bf16),
            pltpu.VMEM((Sq, Dh), bf16),
            pltpu.VMEM((Sq, Dh), bf16),
            pltpu.VMEM((H, Sq, Dh), bf16),
            pltpu.VMEM((S, 2 * Dm), bf16),
            pltpu.VMEM((Dm, 128), f32),
            pltpu.SemaphoreType.DMA((6,)),
            pltpu.SemaphoreType.DMA((2, 3)),
            pltpu.SemaphoreType.DMA((2, 3)),
            pltpu.SemaphoreType.DMA((Sq // 128,)),
        ],
        compiler_params=pltpu.CompilerParams(vmem_limit_bytes=120 * 2**20),
    )(A_x.reshape(S, Dm).T, A_mem0.reshape(M, Dm), A_Wq, A_Wk, A_Wv, A_Wo.transpose(0, 2, 1),
      B_x.reshape(Sq, Dm).T, B_c_kv.reshape(Sq, Dc), B_w_q, B_w_uk, B_w_uv, B_w_o.transpose(0, 2, 1))
    return out.reshape(1, S, 2 * Dm)
```
